```python
import os as _os
_os.environ.setdefault("JAX_PLATFORMS", "cpu")
import jax
import jax.numpy as jnp

def _softmax(x, axis=-1):
    return jax.nn.softmax(x, axis=axis)
def _gelu(x):
    return jax.nn.gelu(x, approximate=True)
def _silu(x):
    return jax.nn.silu(x)
def _sigmoid(x):
    return jax.nn.sigmoid(x)
def _layernorm(x, axis=-1, eps=1e-5):
    m = jnp.mean(x, axis=axis, keepdims=True)
    v = jnp.var(x, axis=axis, keepdims=True)
    return (x - m) / jnp.sqrt(v + eps)
def _scatter_add(tgt, idx, src, axis=0):
    return tgt.at[idx].add(src)
def _segment_sum(src, seg, n):
    return jax.ops.segment_sum(src, seg, n)
class _Rng:
    def __init__(self, key):
        self._k = key
    def _next(self):
        self._k, sub = jax.random.split(self._k)
        return sub
    def normal(self, shape):
        return jax.random.normal(self._next(), shape, dtype=jnp.bfloat16)
    def randint(self, lo, hi, shape):
        return jax.random.randint(self._next(), shape, lo, hi, dtype=jnp.int32)
    def uniform(self, shape, lo=0.0, hi=1.0):
        return jax.random.uniform(self._next(), shape, jnp.bfloat16, lo, hi)
    def permutation(self, n):
        return jax.random.permutation(self._next(), n)


kernel_name = 'concat_heads__gqa_block_cached__sliding_block_cached__decode'

def setup_inputs():
    _rng = _Rng(jax.random.key(int.from_bytes(__import__("os").urandom(4), "little")))
    _w = (lambda a: (lambda t: t.astype(jnp.bfloat16) if jnp.issubdtype(t.dtype, jnp.floating) else t)(jnp.asarray(a)))
    def _A_setup():
        B, Sq, D = 2, 1, 448
        Hq, Hkv, Sk, Dh = 16, 8, 8192, 256
        assert Hq % Hkv == 0, (Hq, Hkv)
        return {
            "x": _w((lambda *s: _rng.normal(s) * 0.8)(B, Sq, D)),
            "k_cache": _w((lambda *s: _rng.normal(s) * 0.8)(B, Hkv, Sk, Dh)),
            "v_cache": _w((lambda *s: _rng.normal(s) * 0.05)(B, Hkv, Sk, Dh)),
            "wq": _w((lambda *s: _rng.normal(s) * 0.8)(D, Hq * Dh) * (D ** -0.5)),
            "wo": _w((lambda *s: _rng.normal(s) * 0.05)(Hq * Dh, D) * ((Hq * Dh) ** -0.5)),
        }
    _A_in = _A_setup()

    def _B_setup():
        B, Sq, D = 2, 1, 448
        Hq, Hkv, Sk, Dh = 16, 8, 8192, 256
        assert Hq % Hkv == 0, (Hq, Hkv)
        return {
            "x": _w((lambda *s: _rng.normal(s) * 0.8)(B, Sq, D)),
            "k_cache": _w((lambda *s: _rng.normal(s) * 0.8)(B, Hkv, Sk, Dh)),
            "v_cache": _w((lambda *s: _rng.normal(s) * 0.05)(B, Hkv, Sk, Dh)),
            "wq": _w((lambda *s: _rng.normal(s) * 0.8)(D, Hq * Dh) * (D ** -0.5)),
            "wo": _w((lambda *s: _rng.normal(s) * 0.05)(Hq * Dh, D) * ((Hq * Dh) ** -0.5)),
        }
    _B_in = _B_setup()

    return {
        "A_x": _A_in["x"],
        "A_k_cache": _A_in["k_cache"],
        "A_v_cache": _A_in["v_cache"],
        "A_wq": _A_in["wq"],
        "A_wo": _A_in["wo"],
        "B_x": _B_in["x"],
        "B_k_cache": _B_in["k_cache"],
        "B_v_cache": _B_in["v_cache"],
        "B_wq": _B_in["wq"],
        "B_wo": _B_in["wo"],
    }

def reference(A_x, A_k_cache, A_v_cache, A_wq, A_wo, B_x, B_k_cache, B_v_cache, B_wq, B_wo):
    def _A_ref(x, k_cache, v_cache, wq, wo):
        B, Sq, D = x.shape
        Hq, Dh = 16, 256
        Hkv = k_cache.shape[1]
        rep = Hq // Hkv
        q = (lambda x, *d: x.transpose(*d))((x @ wq).reshape(B, Sq, Hq, Dh), 0, 2, 1, 3)
        k = jnp.repeat(k_cache, rep, axis=1)
        v = jnp.repeat(v_cache, rep, axis=1)
        scores = jnp.einsum("bhqd,bhkd->bhqk", q, k) * (Dh ** -0.5)
        p = _softmax(scores, axis=-1)
        o = jnp.einsum("bhqk,bhkd->bhqd", p, v)
        return (lambda x, *d: x.transpose(*d))(o, 0, 2, 1, 3).reshape(B, Sq, Hq * Dh) @ wo

    def _B_ref(x, k_cache, v_cache, wq, wo):
        B, Sq, D = x.shape
        Hq, Dh = 16, 256
        Hkv, Sk = k_cache.shape[1], k_cache.shape[2]
        W = min(4096, max(256, Sk // 4))
        rep = Hq // Hkv
        q = (lambda x, *d: x.transpose(*d))((x @ wq).reshape(B, Sq, Hq, Dh), 0, 2, 1, 3)
        k = jnp.repeat(k_cache[:, :, Sk - W:, :], rep, axis=1)
        v = jnp.repeat(v_cache[:, :, Sk - W:, :], rep, axis=1)
        scores = jnp.einsum("bhqd,bhkd->bhqk", q, k) * (Dh ** -0.5)
        p = _softmax(scores, axis=-1)
        o = jnp.einsum("bhqk,bhkd->bhqd", p, v)
        return (lambda x, *d: x.transpose(*d))(o, 0, 2, 1, 3).reshape(B, Sq, Hq * Dh) @ wo

    a = _A_ref(A_x, A_k_cache, A_v_cache, A_wq, A_wo)
    b = _B_ref(B_x, B_k_cache, B_v_cache, B_wq, B_wo)
    return jnp.concatenate([a, b], axis=-1)
```

```python
import jax
import jax.numpy as jnp
import numpy as np
import jax.experimental.pallas as pl
import jax.experimental.pallas.tpu as pltpu

HQ, HKV, DH = 16, 8, 256
REP = HQ // HKV
NT = (((1,), (1,)), ((), ()))


def make(R=128, CH=32, D=2, NS=4, mode="kv", WCH=16, compute=True, semmode="one"):
    def fn(A_x, A_k, A_v, A_wq, A_wo, B_x, B_k, B_v, B_wq, B_wo):
        B, _, DM = A_x.shape
        SK = A_k.shape[2]
        W = min(4096, max(256, SK // 4))
        nA, nB = SK // R, W // R
        TA, TB = B * nA, B * nB
        NP = HKV
        PW = REP * DH
        scale = DH ** -0.5
        neg = float(np.finfo(np.float32).min)

        def kern(ax, bx, ak, av, awq, awo, bk, bv, bwq, bwo, out_ref,
                 kbuf, vbuf, wbuf, qbuf, obuf, ksem, vsem, wsem):

            def issue_w(wa, wb, j):
                col = pl.ds(pl.multiple_of(j * PW, PW), PW)
                for g in range(DM // WCH):
                    rows = pl.ds(g * WCH, WCH)
                    pltpu.make_async_copy(wa.at[rows, col], wbuf.at[j, 0, rows], wsem.at[j]).start(priority=0)
                    pltpu.make_async_copy(wb.at[rows, col], wbuf.at[j, 1, rows], wsem.at[j]).start(priority=1)

            def wait_w(j):
                pltpu.make_async_copy(wbuf.at[j], wbuf.at[j], wsem.at[j]).wait()

            def issue_kv(k_hbm, v_hbm, n, base, u, slot):
                b = u // n
                r0 = base + (u % n) * R

                def cp(isv, h, g, p):
                    src, dst = ((k_hbm, kbuf), (v_hbm, vbuf))[isv]
                    sem = {"one": ksem, "arr": (ksem, vsem)[isv], "prio": (ksem, vsem)[p]}[semmode]
                    rows = pl.ds(pl.multiple_of(r0 + g * CH, CH), CH)
                    pltpu.make_async_copy(src.at[b, h, rows], dst.at[slot, h, pl.ds(g * CH, CH)],
                                          sem.at[slot]).start(priority=p)
                if mode == "kv":
                    for g in range(R // CH):
                        for h in range(HKV):
                            cp(0, h, g, 0)
                            cp(1, h, g, 1)
                elif mode == "alt":
                    for isv in range(2):
                        for g in range(R // CH):
                            for h in range(HKV):
                                cp(isv, h, g, h % 2)
                elif mode == "alt2":
                    for g in range(R // CH):
                        for isv in range(2):
                            for h in range(HKV):
                                cp(isv, h, g, h % 2)

            def wait_kv(slot):
                pltpu.make_async_copy(kbuf.at[slot], kbuf.at[slot], ksem.at[slot]).wait()
                s2 = ksem if semmode == "one" else vsem
                pltpu.make_async_copy(vbuf.at[slot], vbuf.at[slot], s2.at[slot]).wait()

            for j in range(D):
                issue_w(awq, bwq, j)

            row32 = jax.lax.broadcasted_iota(jnp.int32, (B * HQ, DH), 0) % HQ

            def xrows(x_ref):
                x = x_ref[...].astype(jnp.float32)
                return jnp.concatenate(
                    [jnp.broadcast_to(x[b:b + 1], (HQ, DM)) for b in range(B)], axis=0).astype(jnp.bfloat16)
            xs = (xrows(ax), xrows(bx))

            def qproj(j, carry):
                @pl.when(j + D < NP)
                def _():
                    issue_w(awq, bwq, j + D)

                @pl.when(j + D >= NP)
                def _():
                    u = j + D - NP
                    issue_kv(ak, av, nA, 0, u, u % NS)
                wait_w(j)
                new = []
                for p in range(2):
                    q = carry[p]
                    if compute:
                        r = jnp.dot(xs[p], wbuf[j, p], preferred_element_type=jnp.float32)
                        for i in range(REP):
                            q = jnp.where(row32 == j * REP + i, r[:, i * DH:(i + 1) * DH], q)
                    new.append(q)
                return tuple(new)
            z = jnp.zeros((B * HQ, DH), jnp.float32)
            qa, qb = jax.lax.fori_loop(0, NP, qproj, (z, z))
            for p, q in enumerate((qa, qb)):
                for b in range(B):
                    qbuf[p * B + b] = q[b * HQ:(b + 1) * HQ].astype(jnp.bfloat16)

            rowS = jax.lax.broadcasted_iota(jnp.int32, (HQ, R), 0) // REP
            rowO = jax.lax.broadcasted_iota(jnp.int32, (HQ, DH), 0) // REP

            def step(t, carry):
                m, l, acc = carry
                u = t + D

                @pl.when(u < TA)
                def _():
                    issue_kv(ak, av, nA, 0, u, u % NS)

                @pl.when(jnp.logical_and(u >= TA, u < TA + TB))
                def _():
                    issue_kv(bk, bv, nB, SK - W, u - TA, u % NS)

                @pl.when(u >= TA + TB)
                def _():
                    issue_w(awo, bwo, u - TA - TB)
                slot = t % NS
                wait_kv(slot)
                isA = t < TA
                seg = jnp.where(isA, t // nA, B + (t - TA) // nB)
                c = jnp.where(isA, t % nA, (t - TA) % nB)
                last = jnp.where(isA, nA - 1, nB - 1)
                first = c == 0
                m = jnp.where(first, neg, m)
                l = jnp.where(first, 0.0, l)
                acc = jnp.where(first, 0.0, acc)
                if compute:
                    q = qbuf[seg]
                    s = None
                    for h in range(HKV):
                        sh = jax.lax.dot_general(q, kbuf[slot, h], NT, preferred_element_type=jnp.float32)
                        s = sh if s is None else jnp.where(rowS == h, sh, s)
                    s = s * scale
                    m_new = jnp.maximum(m, jnp.max(s, axis=1, keepdims=True))
                    alpha = jnp.exp(m - m_new)
                    p = jnp.exp(s - m_new)
                    ps = p[:, 0:128]
                    for i in range(1, R // 128):
                        ps = ps + p[:, i * 128:(i + 1) * 128]
                    l = l * alpha + ps
                    pb = p.astype(jnp.bfloat16)
                    o = None
                    for h in range(HKV):
                        oh = jnp.dot(pb, vbuf[slot, h], preferred_element_type=jnp.float32)
                        o = oh if o is None else jnp.where(rowO == h, oh, o)
                    acc = acc * alpha + o
                    m = m_new

                @pl.when(c == last)
                def _():
                    obuf[seg] = (acc / jnp.sum(l, axis=1, keepdims=True)).astype(jnp.bfloat16)
                return m, l, acc
            jax.lax.fori_loop(0, TA + TB, step, (jnp.zeros((HQ, 1), jnp.float32),
                                                 jnp.zeros((HQ, 128), jnp.float32),
                                                 jnp.zeros((HQ, DH), jnp.float32)))

            rowT = jax.lax.broadcasted_iota(jnp.int32, (B * HQ, DM), 0) % HQ
            os_ = [jnp.concatenate([obuf[p * B + b] for b in range(B)], axis=0) for p in range(2)]

            def oproj(j, carry):
                @pl.when(j + D < NP)
                def _():
                    issue_w(awo, bwo, j + D)
                wait_w(j)
                new = []
                for p in range(2):
                    tt = carry[p]
                    if compute:
                        for i in range(REP):
                            r = jax.lax.dot_general(os_[p], wbuf[j, p, :, i * DH:(i + 1) * DH], NT,
                                                    preferred_element_type=jnp.float32)
                            tt = jnp.where(rowT == j * REP + i, r, tt)
                    new.append(tt)
                return tuple(new)
            z = jnp.zeros((B * HQ, DM), jnp.float32)
            ta, tb = jax.lax.fori_loop(0, NP, oproj, (z, z))
            res = jnp.concatenate(
                [jnp.concatenate([jnp.sum(tt[b * HQ:(b + 1) * HQ], axis=0, keepdims=True) for b in range(B)], axis=0)
                 for tt in (ta, tb)], axis=1)
            out_ref[...] = res.astype(out_ref.dtype)

        any_ = pl.BlockSpec(memory_space=pl.ANY)
        vmem = pl.BlockSpec(memory_space=pltpu.VMEM)
        out = pl.pallas_call(
            kern,
            in_specs=[vmem, vmem] + [any_] * 8,
            out_specs=vmem,
            out_shape=jax.ShapeDtypeStruct((B, 2 * DM), A_x.dtype),
            scratch_shapes=[
                pltpu.VMEM((NS, HKV, R, DH), jnp.bfloat16),
                pltpu.VMEM((NS, HKV, R, DH), jnp.bfloat16),
                pltpu.VMEM((NP, 2, DM, PW), jnp.bfloat16),
                pltpu.VMEM((2 * B, HQ, DH), jnp.bfloat16),
                pltpu.VMEM((2 * B, HQ, DH), jnp.bfloat16),
                pltpu.SemaphoreType.DMA((NS,)),
                pltpu.SemaphoreType.DMA((NS,)),
                pltpu.SemaphoreType.DMA((NP,)),
            ],
            compiler_params=pltpu.CompilerParams(vmem_limit_bytes=100 * 1024 * 1024, disable_bounds_checks=True),
        )(A_x.reshape(B, DM), B_x.reshape(B, DM), A_k, A_v, A_wq, A_wo.T, B_k, B_v, B_wq, B_wo.T)
        return out.reshape(B, 1, 2 * DM)
    return fn


@jax.jit
def pallas_concat_heads__gqa_block_cached__sliding_block_cached__decode_kernel(
    A_x, A_k_cache, A_v_cache, A_wq, A_wo, B_x, B_k_cache, B_v_cache, B_wq, B_wo,
):
    return make(mode="alt", semmode="arr")(
        A_x, A_k_cache, A_v_cache, A_wq, A_wo, B_x, B_k_cache, B_v_cache, B_wq, B_wo)
```

```python
import jax
import jax.numpy as jnp
import numpy as np
import jax.experimental.pallas as pl
import jax.experimental.pallas.tpu as pltpu

HQ, DH = 16, 256
R = 128
CH = 32
WR, PW = 8, 1024
NS = 2
NT = (((1,), (1,)), ((), ()))


def _queue(k):
    return (k // 2) % 2


def _kv_order():
    fields = [("g", 0), ("h", 0), ("h", 2), ("b", 0), ("h", 1), ("g", 1), ("v", 0)]
    order = []
    for k in range(1 << len(fields)):
        idx = dict(v=0, b=0, h=0, g=0)
        for i, (f, bit) in enumerate(fields):
            idx[f] |= ((k >> i) & 1) << bit
        order.append((idx["v"], idx["b"], idx["h"], idx["g"]))
    return order


@jax.jit
def pallas_concat_heads__gqa_block_cached__sliding_block_cached__decode_kernel(
    A_x: jax.Array,
    A_k_cache: jax.Array,
    A_v_cache: jax.Array,
    A_wq: jax.Array,
    A_wo: jax.Array,
    B_x: jax.Array,
    B_k_cache: jax.Array,
    B_v_cache: jax.Array,
    B_wq: jax.Array,
    B_wo: jax.Array,
):
    B, _, DM = A_x.shape
    _, HKV, SK, _ = A_k_cache.shape
    SKB = B_k_cache.shape[2]
    W = min(4096, max(256, SKB // 4))
    REP = HQ // HKV
    TA, TB = SK // R, W // R
    NP = HQ * DH // PW
    HP = PW // DH
    NR = DM // WR
    assert (B, HKV, R // CH, NP) == (2, 8, 4, 4) and DM % (8 * WR) == 0
    assert SK % R == 0 and W % R == 0 and (SKB - W) % CH == 0 and TA > NP and TB > NP
    scale = DH ** -0.5
    lowest = float(np.finfo(np.float32).min)
    kv_order = _kv_order()
    off4 = [s * (NR // 4) for s in range(4)]
    off7 = [s * 8 for s in range(NR // 8)]
    off8 = [s * (NR // 2) + t * (NR // 4) + u * (NR // 8)
            for u in range(2) for t in range(2) for s in range(2)]

    def kernel(ax, bx, ak, av, awq, awo, bk, bv, bwq, bwo, out_ref,
               kvbuf, wbuf, qbuf, obuf, xbuf, abuf, kvsem, wsem, xsem):
        wq, wo = (awq, bwq), (awo, bwo)

        def issue_w(ws, groups, offs, sem):
            def body(g, carry):
                k = 0
                for group in groups:
                    for off in offs:
                        rows = pl.ds(pl.multiple_of((g + off) * WR, WR), WR)
                        for p, j in group:
                            pltpu.make_async_copy(
                                ws[p].at[rows, pl.ds(j * PW, PW)], wbuf.at[p, j, rows], sem
                            ).start(priority=_queue(k))
                            k += 1
                return carry
            jax.lax.fori_loop(0, NR // len(offs), body, 0)

        def issue_kv(srcs, first_row, slot):
            for k, (v, b, h, g) in enumerate(kv_order):
                rows = pl.ds(pl.multiple_of(first_row + g * CH, CH), CH)
                pltpu.make_async_copy(
                    srcs[v].at[b, h, rows],
                    kvbuf.at[slot, v, b, h, pl.ds(g * CH, CH)],
                    kvsem.at[slot],
                ).start(priority=_queue(k))

        def wait(buf, sem):
            pltpu.make_async_copy(buf, buf, sem).wait()

        def q_proj(p, j):
            r = jnp.dot(xbuf[p], wbuf[p, j], preferred_element_type=jnp.float32)
            for b in range(B):
                for k in range(HP):
                    qbuf[p, b, pl.ds(j * HP + k, 1)] = r[b:b + 1, k * DH:(k + 1) * DH]

        def o_proj(p, j, acc):
            for k in range(HP):
                o = obuf[p, j * HP + k].astype(jnp.bfloat16)
                acc = acc + jax.lax.dot_general(
                    o, wbuf[p, j, :, k * DH:(k + 1) * DH], NT,
                    preferred_element_type=jnp.float32)
            return acc

        x_copies = [pltpu.make_async_copy(x, xbuf.at[p], xsem.at[p])
                    for p, x in enumerate((ax, bx))]
        for c in x_copies:
            c.start()
        issue_w(wq, [[(0, 0), (0, 1), (1, 0), (1, 1)], [(0, 2), (0, 3), (1, 2), (1, 3)]],
                off4, wsem.at[0])
        issue_kv((ak, av), 0, 0)
        for c in x_copies:
            c.wait()
        wait(wbuf, wsem.at[0])

        def q_a(j, carry):
            q_proj(0, j)
            return carry
        jax.lax.fori_loop(0, NP, q_a, 0)

        head_s = jax.lax.broadcasted_iota(jnp.int32, (HQ, R), 0) // REP
        head_o = jax.lax.broadcasted_iota(jnp.int32, (HQ, DH), 0) // REP

        def step(t, carry):
            u = t + 1

            @pl.when(u < TA)
            def _():
                issue_kv((ak, av), u * R, u % NS)

            @pl.when(jnp.logical_and(u >= TA, u < TA + TB))
            def _():
                issue_kv((bk, bv), SKB - W + (u - TA) * R, u % NS)

            @pl.when(u == TA + TB)
            def _():
                issue_w(wo, [[(1, 0), (1, 1)]], off8, wsem.at[2])

            @pl.when(t == NP)
            def _():
                issue_w(wo, [[(0, 0), (0, 1)], [(0, 2), (0, 3)]], off8, wsem.at[1])

            slot = t % NS
            wait(kvbuf.at[slot], kvsem.at[slot])

            @pl.when(t < NP)
            def _():
                q_proj(1, t)

            @pl.when(t == TA)
            def _():
                wait(wbuf.at[0], wsem.at[1])
                abuf[...] = jnp.zeros_like(abuf)

            @pl.when(jnp.logical_and(t >= TA, t < TA + NP))
            def _():
                abuf[...] = o_proj(0, t - TA, abuf[...])

            @pl.when(t == TA + NP)
            def _():
                out_ref[:, 0:DM] = abuf[...].astype(out_ref.dtype)

            blk = (t >= TA).astype(jnp.int32)
            first = jnp.logical_or(t == 0, t == TA)
            last = jnp.logical_or(t == TA - 1, t == TA + TB - 1)
            new = []
            for b in range(B):
                m, l, acc = carry[b]
                m = jnp.where(first, lowest, m)
                l = jnp.where(first, 0.0, l)
                acc = jnp.where(first, 0.0, acc)
                q = qbuf[blk, b].astype(jnp.bfloat16)
                s = None
                for h in range(HKV):
                    sh = jax.lax.dot_general(
                        q, kvbuf[slot, 0, b, h], NT, preferred_element_type=jnp.float32)
                    s = sh if s is None else jnp.where(head_s == h, sh, s)
                s = s * scale
                m_new = jnp.maximum(m, jnp.max(s, axis=1, keepdims=True))
                alpha = jnp.exp(m - m_new)
                p = jnp.exp(s - m_new)
                l = l * alpha + p
                p = p.astype(jnp.bfloat16)
                o = None
                for h in range(HKV):
                    oh = jnp.dot(p, kvbuf[slot, 1, b, h], preferred_element_type=jnp.float32)
                    o = oh if o is None else jnp.where(head_o == h, oh, o)
                new.append((m_new, l, acc * alpha + o))

            @pl.when(last)
            def _():
                for b in range(B):
                    _, l, acc = new[b]
                    o = acc / jnp.sum(l, axis=1, keepdims=True)
                    for r in range(HQ):
                        obuf[blk, r, b:b + 1] = o[r:r + 1]

            return tuple(new)

        init = tuple((jnp.zeros((HQ, 1), jnp.float32),
                      jnp.zeros((HQ, R), jnp.float32),
                      jnp.zeros((HQ, DH), jnp.float32)) for _ in range(B))
        jax.lax.fori_loop(0, TA + TB, step, init)

        issue_w(wo, [[(1, 2)]], off8, wsem.at[3])
        issue_w(wo, [[(1, 3)]], off7, wsem.at[4])
        wait(wbuf.at[1, 0:2], wsem.at[2])
        acc = jax.lax.fori_loop(0, 2, lambda j, a: o_proj(1, j, a),
                                jnp.zeros((B, DM), jnp.float32))
        wait(wbuf.at[1, 2], wsem.at[3])
        acc = o_proj(1, 2, acc)
        wait(wbuf.at[1, 3], wsem.at[4])
        out_ref[:, DM:2 * DM] = o_proj(1, 3, acc).astype(out_ref.dtype)

    out = pl.pallas_call(
        kernel,
        in_specs=[pl.BlockSpec(memory_space=pl.ANY)] * 10,
        out_specs=pl.BlockSpec(memory_space=pltpu.VMEM),
        out_shape=jax.ShapeDtypeStruct((B, 2 * DM), A_x.dtype),
        scratch_shapes=[
            pltpu.VMEM((NS, 2, B, HKV, R, DH), A_k_cache.dtype),
            pltpu.VMEM((2, NP, DM, PW), A_wq.dtype),
            pltpu.VMEM((2, B, HQ, DH), jnp.float32),
            pltpu.VMEM((2, HQ, B, DH), jnp.float32),
            pltpu.VMEM((2, B, DM), A_x.dtype),
            pltpu.VMEM((B, DM), jnp.float32),
            pltpu.SemaphoreType.DMA((NS,)),
            pltpu.SemaphoreType.DMA((5,)),
            pltpu.SemaphoreType.DMA((2,)),
        ],
        compiler_params=pltpu.CompilerParams(
            vmem_limit_bytes=32 * 1024 * 1024, disable_bounds_checks=True),
    )(A_x.reshape(B, DM), B_x.reshape(B, DM),
      A_k_cache, A_v_cache, A_wq, A_wo.T,
      B_k_cache, B_v_cache, B_wq, B_wo.T)
    return out.reshape(B, 1, 2 * DM)
```

```python
import jax
import jax.numpy as jnp
import numpy as np
import jax.experimental.pallas as pl
import jax.experimental.pallas.tpu as pltpu

HQ, DH = 16, 256
R = 128
CH = 32
WR, PW = 8, 1024
NS = 2
NT = (((1,), (1,)), ((), ()))


def _queue(k):
    return (k // 2) % 2


def _kv_order():
    fields = [("g", 0), ("h", 0), ("h", 2), ("b", 0), ("h", 1), ("g", 1), ("v", 0)]
    order = []
    for k in range(1 << len(fields)):
        idx = dict(v=0, b=0, h=0, g=0)
        for i, (f, bit) in enumerate(fields):
            idx[f] |= ((k >> i) & 1) << bit
        order.append((idx["v"], idx["b"], idx["h"], idx["g"]))
    return order


@jax.jit
def pallas_concat_heads__gqa_block_cached__sliding_block_cached__decode_kernel(
    A_x: jax.Array,
    A_k_cache: jax.Array,
    A_v_cache: jax.Array,
    A_wq: jax.Array,
    A_wo: jax.Array,
    B_x: jax.Array,
    B_k_cache: jax.Array,
    B_v_cache: jax.Array,
    B_wq: jax.Array,
    B_wo: jax.Array,
):
    B, _, DM = A_x.shape
    _, HKV, SK, _ = A_k_cache.shape
    SKB = B_k_cache.shape[2]
    W = min(4096, max(256, SKB // 4))
    REP = HQ // HKV
    TA, TB = SK // R, W // R
    NP = HQ * DH // PW
    HP = PW // DH
    NR = DM // WR
    assert (B, HKV, R // CH, NP) == (2, 8, 4, 4) and DM % (8 * WR) == 0
    assert SK % R == 0 and W % R == 0 and (SKB - W) % CH == 0 and TA > NP and TB > NP
    scale = DH ** -0.5
    lowest = float(np.finfo(np.float32).min)
    kv_order = _kv_order()
    off4 = [s * (NR // 4) for s in range(4)]
    off8 = [s * (NR // 2) + t * (NR // 4) + u * (NR // 8)
            for u in range(2) for t in range(2) for s in range(2)]

    def kernel(ax, bx, ak, av, awq, awo, bk, bv, bwq, bwo, out_ref,
               kvbuf, wbuf, qbuf, obuf, xbuf, abuf, kvsem, wsem, xsem):
        wq, wo = (awq, bwq), (awo, bwo)

        def issue_w(ws, groups, offs, sem):
            def body(g, carry):
                k = 0
                for group in groups:
                    for off in offs:
                        rows = pl.ds(pl.multiple_of((g + off) * WR, WR), WR)
                        for p, j in group:
                            pltpu.make_async_copy(
                                ws[p].at[rows, pl.ds(j * PW, PW)], wbuf.at[p, j, rows], sem
                            ).start(priority=_queue(k))
                            k += 1
                return carry
            jax.lax.fori_loop(0, NR // len(offs), body, 0)

        def issue_kv(srcs, first_row, slot):
            for k, (v, b, h, g) in enumerate(kv_order):
                rows = pl.ds(pl.multiple_of(first_row + g * CH, CH), CH)
                pltpu.make_async_copy(
                    srcs[v].at[b, h, rows],
                    kvbuf.at[slot, v, b, h, pl.ds(g * CH, CH)],
                    kvsem.at[slot],
                ).start(priority=_queue(k))

        def wait(buf, sem):
            pltpu.make_async_copy(buf, buf, sem).wait()

        def q_proj(p, j):
            r = jnp.dot(xbuf[p], wbuf[p, j], preferred_element_type=jnp.float32)
            for b in range(B):
                for k in range(HP):
                    qbuf[p, b, pl.ds(j * HP + k, 1)] = r[b:b + 1, k * DH:(k + 1) * DH]

        def o_proj(p, j, acc, heads=range(HP)):
            for k in heads:
                o = obuf[p, j * HP + k].astype(jnp.bfloat16)
                acc = acc + jax.lax.dot_general(
                    o, wbuf[p, j, :, k * DH:(k + 1) * DH], NT,
                    preferred_element_type=jnp.float32)
            return acc

        x_copies = [pltpu.make_async_copy(x, xbuf.at[p], xsem.at[p])
                    for p, x in enumerate((ax, bx))]
        for c in x_copies:
            c.start()
        issue_w(wq, [[(0, 0), (0, 1), (1, 0), (1, 1)], [(0, 2), (0, 3), (1, 2), (1, 3)]],
                off4, wsem.at[0])
        issue_kv((ak, av), 0, 0)
        for c in x_copies:
            c.wait()
        wait(wbuf, wsem.at[0])

        def q_a(j, carry):
            q_proj(0, j)
            return carry
        jax.lax.fori_loop(0, NP, q_a, 0)

        head_s = jax.lax.broadcasted_iota(jnp.int32, (HQ, R), 0) // REP
        head_o = jax.lax.broadcasted_iota(jnp.int32, (HQ, DH), 0) // REP

        def step(t, carry):
            u = t + 1

            @pl.when(u < TA)
            def _():
                issue_kv((ak, av), u * R, u % NS)

            @pl.when(jnp.logical_and(u >= TA, u < TA + TB))
            def _():
                issue_kv((bk, bv), SKB - W + (u - TA) * R, u % NS)

            @pl.when(u == TA + TB)
            def _():
                issue_w(wo, [[(1, 0), (1, 1)]], off8, wsem.at[2])

            @pl.when(t == NP)
            def _():
                issue_w(wo, [[(0, 0), (0, 1)], [(0, 2), (0, 3)]], off8, wsem.at[1])

            slot = t % NS
            wait(kvbuf.at[slot], kvsem.at[slot])

            @pl.when(t < NP)
            def _():
                q_proj(1, t)

            @pl.when(t == TA)
            def _():
                wait(wbuf.at[0], wsem.at[1])
                abuf[...] = jnp.zeros_like(abuf)

            @pl.when(jnp.logical_and(t >= TA, t < TA + NP))
            def _():
                abuf[...] = o_proj(0, t - TA, abuf[...])

            @pl.when(t == TA + NP)
            def _():
                out_ref[:, 0:DM] = abuf[...].astype(out_ref.dtype)

            blk = (t >= TA).astype(jnp.int32)
            first = jnp.logical_or(t == 0, t == TA)
            last = jnp.logical_or(t == TA - 1, t == TA + TB - 1)
            new = []
            for b in range(B):
                m, l, acc = carry[b]
                m = jnp.where(first, lowest, m)
                l = jnp.where(first, 0.0, l)
                acc = jnp.where(first, 0.0, acc)
                q = qbuf[blk, b].astype(jnp.bfloat16)
                s = None
                for h in range(HKV):
                    sh = jax.lax.dot_general(
                        q, kvbuf[slot, 0, b, h], NT, preferred_element_type=jnp.float32)
                    s = sh if s is None else jnp.where(head_s == h, sh, s)
                s = s * scale
                m_new = jnp.maximum(m, jnp.max(s, axis=1, keepdims=True))
                alpha = jnp.exp(m - m_new)
                p = jnp.exp(s - m_new)
                l = l * alpha + p
                p = p.astype(jnp.bfloat16)
                o = None
                for h in range(HKV):
                    oh = jnp.dot(p, kvbuf[slot, 1, b, h], preferred_element_type=jnp.float32)
                    o = oh if o is None else jnp.where(head_o == h, oh, o)
                new.append((m_new, l, acc * alpha + o))

            @pl.when(last)
            def _():
                for b in range(B):
                    _, l, acc = new[b]
                    o = acc / jnp.sum(l, axis=1, keepdims=True)
                    for r in range(HQ):
                        obuf[blk, r, b:b + 1] = o[r:r + 1]

            return tuple(new)

        init = tuple((jnp.zeros((HQ, 1), jnp.float32),
                      jnp.zeros((HQ, R), jnp.float32),
                      jnp.zeros((HQ, DH), jnp.float32)) for _ in range(B))
        jax.lax.fori_loop(0, TA + TB, step, init)

        issue_w(wo, [[(1, 2)]], off8, wsem.at[3])
        half = PW // 2
        tail_rows = [pl.ds((s * 4 + g) * 2 * WR, 2 * WR)
                     for g in range(4) for s in range(NR // 8)]
        for i in range(0, len(tail_rows), 2):
            for c in range(2):
                for rows in tail_rows[i:i + 2]:
                    pltpu.make_async_copy(
                        bwo.at[rows, pl.ds(3 * PW + c * half, half)],
                        wbuf.at[1, 3, rows, pl.ds(c * half, half)],
                        wsem.at[4 + c],
                    ).start(priority=c)
        wait(wbuf.at[1, 0:2], wsem.at[2])
        acc = jax.lax.fori_loop(0, 2, lambda j, a: o_proj(1, j, a),
                                jnp.zeros((B, DM), jnp.float32))
        wait(wbuf.at[1, 2], wsem.at[3])
        acc = o_proj(1, 2, acc)
        for c in range(2):
            wait(wbuf.at[1, 3, :, pl.ds(c * half, half)], wsem.at[4 + c])
            acc = o_proj(1, 3, acc, range(c * HP // 2, (c + 1) * HP // 2))
        out_ref[:, DM:2 * DM] = acc.astype(out_ref.dtype)

    out = pl.pallas_call(
        kernel,
        in_specs=[pl.BlockSpec(memory_space=pl.ANY)] * 10,
        out_specs=pl.BlockSpec(memory_space=pltpu.VMEM),
        out_shape=jax.ShapeDtypeStruct((B, 2 * DM), A_x.dtype),
        scratch_shapes=[
            pltpu.VMEM((NS, 2, B, HKV, R, DH), A_k_cache.dtype),
            pltpu.VMEM((2, NP, DM, PW), A_wq.dtype),
            pltpu.VMEM((2, B, HQ, DH), jnp.float32),
            pltpu.VMEM((2, HQ, B, DH), jnp.float32),
            pltpu.VMEM((2, B, DM), A_x.dtype),
            pltpu.VMEM((B, DM), jnp.float32),
            pltpu.SemaphoreType.DMA((NS,)),
            pltpu.SemaphoreType.DMA((6,)),
            pltpu.SemaphoreType.DMA((2,)),
        ],
        compiler_params=pltpu.CompilerParams(
            vmem_limit_bytes=32 * 1024 * 1024, disable_bounds_checks=True),
    )(A_x.reshape(B, DM), B_x.reshape(B, DM),
      A_k_cache, A_v_cache, A_wq, A_wo.T,
      B_k_cache, B_v_cache, B_wq, B_wo.T)
    return out.reshape(B, 1, 2 * DM)
```
